```python
import os as _os
_os.environ.setdefault("JAX_PLATFORMS", "cpu")
import jax
import jax.numpy as jnp

def _softmax(x, axis=-1):
    return jax.nn.softmax(x, axis=axis)
def _gelu(x):
    return jax.nn.gelu(x, approximate=True)
def _silu(x):
    return jax.nn.silu(x)
def _sigmoid(x):
    return jax.nn.sigmoid(x)
def _layernorm(x, axis=-1, eps=1e-5):
    m = jnp.mean(x, axis=axis, keepdims=True)
    v = jnp.var(x, axis=axis, keepdims=True)
    return (x - m) / jnp.sqrt(v + eps)
def _scatter_add(tgt, idx, src, axis=0):
    return tgt.at[idx].add(src)
def _segment_sum(src, seg, n):
    return jax.ops.segment_sum(src, seg, n)
class _Rng:
    def __init__(self, key):
        self._k = key
    def _next(self):
        self._k, sub = jax.random.split(self._k)
        return sub
    def normal(self, shape):
        return jax.random.normal(self._next(), shape, dtype=jnp.bfloat16)
    def randint(self, lo, hi, shape):
        return jax.random.randint(self._next(), shape, lo, hi, dtype=jnp.int32)
    def uniform(self, shape, lo=0.0, hi=1.0):
        return jax.random.uniform(self._next(), shape, jnp.bfloat16, lo, hi)
    def permutation(self, n):
        return jax.random.permutation(self._next(), n)


kernel_name = 'standalone__gqa_block_cached__sampling'

def setup_inputs():
    _rng = _Rng(jax.random.key(int.from_bytes(__import__("os").urandom(4), "little")))
    _w = (lambda a: (lambda t: t.astype(jnp.bfloat16) if jnp.issubdtype(t.dtype, jnp.floating) else t)(jnp.asarray(a)))
    B, Sq, D = 32, 16, 1024
    Hq, Hkv, Sk, Dh = 32, 4, 2048, 128
    assert Hq % Hkv == 0, (Hq, Hkv)
    return {
        "x": _w((lambda *s: _rng.normal(s) * 0.8)(B, Sq, D)),
        "k_cache": _w((lambda *s: _rng.normal(s) * 0.8)(B, Hkv, Sk, Dh)),
        "v_cache": _w((lambda *s: _rng.normal(s) * 0.05)(B, Hkv, Sk, Dh)),
        "wq": _w((lambda *s: _rng.normal(s) * 0.8)(D, Hq * Dh) * (D ** -0.5)),
        "wo": _w((lambda *s: _rng.normal(s) * 0.05)(Hq * Dh, D) * ((Hq * Dh) ** -0.5)),
    }

def reference(x, k_cache, v_cache, wq, wo):
    B, Sq, D = x.shape
    Hq, Dh = 32, 128
    Hkv = k_cache.shape[1]
    rep = Hq // Hkv
    q = (lambda x, *d: x.transpose(*d))((x @ wq).reshape(B, Sq, Hq, Dh), 0, 2, 1, 3)
    k = jnp.repeat(k_cache, rep, axis=1)
    v = jnp.repeat(v_cache, rep, axis=1)
    scores = jnp.einsum("bhqd,bhkd->bhqk", q, k) * (Dh ** -0.5)
    p = _softmax(scores, axis=-1)
    o = jnp.einsum("bhqk,bhkd->bhqd", p, v)
    return (lambda x, *d: x.transpose(*d))(o, 0, 2, 1, 3).reshape(B, Sq, Hq * Dh) @ wo
```

```python
import functools
import math

import jax
import jax.numpy as jnp
import numpy as np
from jax import lax
from jax.experimental import pallas as pl
from jax.experimental.pallas import tpu as pltpu

B, SQ, D = 32, 16, 1024
HQ, HKV, SK, DH = 32, 4, 2048, 128
REP = HQ // HKV
RB = 8
NR = B // RB
NRHO = NR * HKV
NBLK = B * HKV
BF = jnp.bfloat16
F32 = jnp.float32
QSCALE = float(DH ** -0.5 * math.log2(math.e))


def make_kernel(cfg):
    LOOK = cfg.get("look", 8)
    NBUF = cfg.get("nbuf", 16)
    chunks = cfg.get("chunks", [192] * 10 + [128])
    assert sum(chunks) == SK
    order = cfg.get("order", "dma,kw,vw,qk,qp,sm,pv,op")

    def kernel(x_hbm, k_hbm, v_hbm, wq_hbm, wo_hbm, out_hbm,
               x_s, wq_s, wo_s, kbuf, vbuf, q_s, o_s, acc_s, out_s,
               sem_k, sem_v, sem_x, sem_wq, sem_wo, sem_out):

        def kv_start(n):
            g = n // B
            b = n % B
            slot = n % NBUF
            off = 0
            for r in chunks:
                pltpu.make_async_copy(k_hbm.at[b, g, pl.ds(off, r)], kbuf.at[slot, pl.ds(off, r)],
                                      sem_k.at[slot]).start(priority=0)
                pltpu.make_async_copy(v_hbm.at[b, g, pl.ds(off, r)], vbuf.at[slot, pl.ds(off, r)],
                                      sem_v.at[slot]).start(priority=1)
                off += r

        def k_wait(n):
            slot = n % NBUF
            pltpu.make_async_copy(kbuf.at[slot], kbuf.at[slot], sem_k.at[slot]).wait()

        def v_wait(n):
            slot = n % NBUF
            pltpu.make_async_copy(vbuf.at[slot], vbuf.at[slot], sem_v.at[slot]).wait()

        def wq_copies(g):
            c0 = pl.multiple_of(g * 1024, 1024) if not isinstance(g, int) else g * 1024
            return [pltpu.make_async_copy(wq_hbm.at[pl.ds(h * 512, 512), pl.ds(c0, 1024)],
                                          wq_s.at[pl.ds(h * 512, 512), pl.ds(c0, 1024)],
                                          sem_wq.at[h]) for h in range(2)]

        def wo_copies(g):
            r0 = g * 1024
            res = []
            for h in range(2):
                rr = r0 + h * 512
                if not isinstance(g, int):
                    rr = pl.multiple_of(rr, 512)
                res.append(pltpu.make_async_copy(wo_hbm.at[pl.ds(rr, 512)], wo_s.at[pl.ds(rr, 512)],
                                                 sem_wo.at[h]))
            return res

        def x_copies():
            return [pltpu.make_async_copy(x_hbm.at[pl.ds(0, 128)], x_s.at[pl.ds(0, 128)], sem_x.at[0]),
                    pltpu.make_async_copy(x_hbm.at[pl.ds(128, 384)], x_s.at[pl.ds(128, 384)], sem_x.at[1])]

        def out_copy(r):
            r0 = r * 128 if isinstance(r, int) else pl.multiple_of(r * 128, 128)
            return pltpu.make_async_copy(out_s.at[pl.ds(r0, 128)], out_hbm.at[pl.ds(r0, 128)], sem_out.at[r])

        def mo(v, m):
            return v if isinstance(v, int) else pl.multiple_of(v, m)

        def q_piece(rho, j):
            g = rho // NR
            r = rho % NR
            xs = x_s[pl.ds(mo(r * 128, 128), 128), :]
            w = wq_s[:, pl.ds(mo((g * REP + j) * 128, 128), 128)]
            q = jnp.dot(xs, w, preferred_element_type=F32) * QSCALE
            q = q.astype(BF)
            par = rho % 2
            for bl in range(RB):
                q_s[par, bl, pl.ds(mo(j * 16, 16), 16), :] = q[bl * 16:(bl + 1) * 16]

        def out_piece(rho, j):
            g = rho // NR
            r = rho % NR
            par = rho % 2
            c0 = mo(j * 128, 128)
            w = wo_s[pl.ds(mo(g * 1024, 1024), 1024), pl.ds(c0, 128)]
            res = jnp.dot(o_s[par], w, preferred_element_type=F32)
            rows = pl.ds(mo(r * 128, 128), 128)
            res = res + acc_s[rows, pl.ds(c0, 128)]
            acc_s[rows, pl.ds(c0, 128)] = res
            out_s[rows, pl.ds(c0, 128)] = res.astype(BF)

        def qk(rho, j, n):
            slot = n % NBUF
            q = q_s[rho % 2, j]
            return lax.dot_general(q, kbuf[slot], (((1,), (1,)), ((), ())), preferred_element_type=F32)

        def softmax(s):
            m = jnp.max(s, axis=-1, keepdims=True)
            p = jnp.exp2(s - m)
            l = jnp.sum(p, axis=-1, keepdims=True)
            return p.astype(BF), l

        def pv(rho, j, n, p, l):
            slot = n % NBUF
            o = jnp.dot(p, vbuf[slot], preferred_element_type=F32)
            o = (o * (1.0 / l)).astype(BF)
            par = rho % 2
            for h in range(REP):
                o_s[par, pl.ds(mo(j * 16, 16), 16), h * 128:(h + 1) * 128] = o[h * 16:(h + 1) * 16]

        def body(rho, j, do_q, do_out, do_dma):
            n = rho * RB + j
            st = {}
            for op in order.split(","):
                if op == "dma":
                    if do_dma:
                        kv_start(n + LOOK)
                elif op == "kw":
                    k_wait(n)
                elif op == "vw":
                    v_wait(n)
                elif op == "qk":
                    st["s"] = qk(rho, j, n)
                elif op == "sm":
                    st["p"], st["l"] = softmax(st["s"])
                elif op == "pv":
                    pv(rho, j, n, st["p"], st["l"])
                elif op == "qp":
                    if do_q:
                        q_piece(rho + 1, j)
                elif op == "op":
                    if do_out:
                        out_piece(rho - 1, j)

        xc = x_copies()
        xc[0].start(priority=0)
        w0 = wq_copies(0)
        w0[0].start(priority=0)
        w0[1].start(priority=1)
        xc[1].start(priority=1)
        for n in range(min(2, LOOK)):
            kv_start(n)
        wo0 = wo_copies(0)
        wo0[0].start(priority=0)
        wo0[1].start(priority=1)
        for n in range(2, LOOK):
            kv_start(n)
        acc_s[...] = jnp.zeros(acc_s.shape, F32)
        xc[0].wait()
        w0[0].wait()
        w0[1].wait()

        @pl.loop(0, RB)
        def _(j):
            q_piece(0, j)

        xc[1].wait()

        assert LOOK <= RB
        w1 = wq_copies(1)
        w1[0].start(priority=0)
        w1[1].start(priority=1)

        @pl.loop(0, RB)
        def _(j):
            body(0, j, True, False, True)

        wo0[0].wait()
        wo0[1].wait()

        @pl.loop(1, NRHO - 1)
        def _(rho):
            @pl.when(jnp.logical_and(rho % NR == 3, rho < 12))
            def _():
                for c in wq_copies((rho + 1) // NR):
                    c.wait()

            @pl.when(jnp.logical_and(rho % NR == 1, rho > 1))
            def _():
                for c in wo_copies((rho - 1) // NR):
                    c.wait()

            @pl.when(jnp.logical_and(rho % NR == 2, rho < 12))
            def _():
                cs = wo_copies(rho // NR + 1)
                cs[0].start(priority=0)
                cs[1].start(priority=1)

            @pl.when(jnp.logical_and(rho % NR == 0, rho < 12))
            def _():
                cs = wq_copies(rho // NR + 1)
                cs[0].start(priority=0)
                cs[1].start(priority=1)

            @pl.when(rho == 14)
            def _():
                out_copy(0).start()

            if LOOK == RB:
                @pl.loop(0, RB)
                def _(j):
                    body(rho, j, True, True, True)
            else:
                @pl.loop(0, RB)
                def _(j):
                    body(rho, j, True, True, True)

        out_copy(1).start()

        if LOOK == RB:
            @pl.loop(0, RB)
            def _(j):
                body(NRHO - 1, j, False, True, False)
        else:
            @pl.loop(0, RB - LOOK)
            def _(j):
                body(NRHO - 1, j, False, True, True)

            @pl.loop(RB - LOOK, RB)
            def _(j):
                body(NRHO - 1, j, False, True, False)

        out_copy(2).start()

        @pl.loop(0, RB)
        def _(j):
            out_piece(NRHO - 1, j)

        out_copy(3).start()
        for r in range(NR):
            out_copy(r).wait()

    scratch = [
        pltpu.VMEM((B * SQ, D), BF),
        pltpu.VMEM((D, HQ * DH), BF),
        pltpu.VMEM((HQ * DH, D), BF),
        pltpu.VMEM((NBUF, SK, DH), BF),
        pltpu.VMEM((NBUF, SK, DH), BF),
        pltpu.VMEM((2, RB, REP * SQ, DH), BF),
        pltpu.VMEM((2, RB * SQ, REP * DH), BF),
        pltpu.VMEM((B * SQ, D), F32),
        pltpu.VMEM((B * SQ, D), BF),
        pltpu.SemaphoreType.DMA((NBUF,)),
        pltpu.SemaphoreType.DMA((NBUF,)),
        pltpu.SemaphoreType.DMA((2,)),
        pltpu.SemaphoreType.DMA((2,)),
        pltpu.SemaphoreType.DMA((2,)),
        pltpu.SemaphoreType.DMA((NR,)),
    ]
    return pl.pallas_call(
        kernel,
        out_shape=jax.ShapeDtypeStruct((B * SQ, D), BF),
        in_specs=[pl.BlockSpec(memory_space=pl.ANY)] * 5,
        out_specs=pl.BlockSpec(memory_space=pl.ANY),
        scratch_shapes=scratch,
        compiler_params=pltpu.CompilerParams(vmem_limit_bytes=100 * 1024 * 1024, flags=cfg.get("flags"), disable_bounds_checks=cfg.get("nobc", True)),
        name=cfg.get("name", "k1"),
    )


def build(cfg):
    call = make_kernel(cfg)

    def fn(x, k_cache, v_cache, wq, wo):
        out = call(x.reshape(B * SQ, D), k_cache, v_cache, wq, wo)
        return out.reshape(B, SQ, D)
    return fn


_fn = build(dict(order="kw,vw,qk,op,qp,sm,pv,dma", name="gqa_block_cached"))


@jax.jit
def pallas_standalone__gqa_block_cached__sampling_kernel(x, k_cache, v_cache, wq, wo):
    return _fn(x, k_cache, v_cache, wq, wo)
```

```python
import math

import jax
import jax.numpy as jnp
from jax import lax
from jax.experimental import pallas as pl
from jax.experimental.pallas import tpu as pltpu

B, SQ, D = 32, 16, 1024
HQ, HKV, SK, DH = 32, 4, 2048, 128
REP = HQ // HKV
GW = REP * DH
RB = 4
RR = RB * SQ
NR = B // RB
NPH = NR * HKV
NBLK = B * HKV
PW = GW // RB
HP = PW // DH

K_AHEAD = 3
V_AHEAD = 5
NKB = K_AHEAD + 1
NVB = V_AHEAD + 1
KV_CHUNKS = (192,) * 10 + (128,)

BF = jnp.bfloat16
F32 = jnp.float32
QSCALE = float(DH ** -0.5 * math.log2(math.e))

assert sum(KV_CHUNKS) == SK and NKB == 4 and RB == 4


def _aligned(v, m):
    return v if isinstance(v, int) else pl.multiple_of(v, m)


def _kernel(x_hbm, k_hbm, v_hbm, wq_hbm, wo_hbm, out_hbm,
            x_s, wq_s, wo_s, kbuf, vbuf, q_s, p_s, il_s, o_s, acc_s, out_s,
            sem_k, sem_v, sem_a, sem_b, sem_c):

    def block_start(hbm, buf, sem, n, ring, queue):
        off = 0
        for rows in KV_CHUNKS:
            pltpu.make_async_copy(hbm.at[n % B, n // B, pl.ds(off, rows)],
                                  buf.at[n % ring, pl.ds(off, rows)],
                                  sem.at[n % ring]).start(priority=queue)
            off += rows

    def block_wait(buf, sem, n, ring):
        pltpu.make_async_copy(buf.at[n % ring], buf.at[n % ring], sem.at[n % ring]).wait()

    def k_start(n):
        block_start(k_hbm, kbuf, sem_k, n, NKB, 0)

    def v_start(n):
        block_start(v_hbm, vbuf, sem_v, n, NVB, 1)

    def k_wait(n):
        block_wait(kbuf, sem_k, n, NKB)

    def v_wait(n):
        block_wait(vbuf, sem_v, n, NVB)

    def wq_copies(g):
        c0 = _aligned(g * GW, GW)
        return [pltpu.make_async_copy(wq_hbm.at[pl.ds(h * 512, 512), pl.ds(c0, GW)],
                                      wq_s.at[pl.ds(h * 512, 512), pl.ds(c0, GW)], sem_a)
                for h in range(2)]

    def wo_copies(g):
        return [pltpu.make_async_copy(wo_hbm.at[pl.ds(_aligned(g * GW + h * 512, 512), 512)],
                                      wo_s.at[pl.ds(_aligned(g * GW + h * 512, 512), 512)], sem_c)
                for h in range(2)]

    def start_split(copies):
        copies[0].start(priority=0)
        copies[1].start(priority=1)

    def wait_all(copies):
        for c in copies:
            c.wait()

    def out_copy(r0, rows):
        return pltpu.make_async_copy(out_s.at[pl.ds(r0, rows)], out_hbm.at[pl.ds(r0, rows)], sem_b)

    def q_piece(ph, j):
        g, r = ph // NR, ph % NR
        xs = x_s[pl.ds(_aligned(r * RR, RR), RR), :]
        w = wq_s[:, pl.ds(_aligned(g * GW + j * PW, PW), PW)]
        q = (jnp.dot(xs, w, preferred_element_type=F32) * QSCALE).astype(BF)
        for bl in range(RB):
            for t in range(HP):
                q_s[ph % 2, bl, pl.ds(_aligned((j * HP + t) * SQ, SQ), SQ), :] = (
                    q[bl * SQ:(bl + 1) * SQ, t * DH:(t + 1) * DH])

    def scores(ph, j):
        return lax.dot_general(q_s[ph % 2, j], kbuf[(ph * RB + j) % NKB],
                               (((1,), (1,)), ((), ())), preferred_element_type=F32)

    def softmax(ph, j, s):
        m = jnp.max(s, axis=-1, keepdims=True)
        p = jnp.exp2(s - m)
        l = jnp.sum(p, axis=-1, keepdims=True)
        p_s[ph % 2, j] = p.astype(BF)
        il_s[ph % 2, j] = jnp.broadcast_to(1.0 / l, (GW // DH * SQ, DH))

    def attend(ph, j):
        o = jnp.dot(p_s[ph % 2, j], vbuf[(ph * RB + j) % NVB], preferred_element_type=F32)
        o = (o * il_s[ph % 2, j]).astype(BF)
        for h in range(REP):
            o_s[ph % 2, pl.ds(_aligned(j * SQ, SQ), SQ), h * DH:(h + 1) * DH] = o[h * SQ:(h + 1) * SQ]

    def out_piece(ph, j, width=PW):
        g, r = ph // NR, ph % NR
        cols = pl.ds(_aligned(j * width, width), width)
        rows = pl.ds(_aligned(r * RR, RR), RR)
        res = jnp.dot(o_s[ph % 2], wo_s[pl.ds(_aligned(g * GW, GW), GW), cols],
                      preferred_element_type=F32) + acc_s[rows, cols]
        acc_s[rows, cols] = res
        out_s[rows, cols] = res.astype(BF)

    def step(ph, j, v_side=True, out_side=True):
        n = ph * RB + j
        k_wait(n + RB)
        if v_side:
            v_wait(n)
            attend(ph, j)
        s = scores(ph + 1, j)
        if out_side:
            out_piece(ph - 1, j)
        q_piece(ph + 2, j)
        softmax(ph + 1, j, s)
        k_start(n + RB + K_AHEAD)
        v_start(n + V_AHEAD)

    x_head = pltpu.make_async_copy(x_hbm.at[pl.ds(0, 2 * RR)], x_s.at[pl.ds(0, 2 * RR)], sem_a)
    x_rest = pltpu.make_async_copy(x_hbm.at[pl.ds(2 * RR, B * SQ - 2 * RR)],
                                   x_s.at[pl.ds(2 * RR, B * SQ - 2 * RR)], sem_b)
    x_head.start(priority=0)
    for c in wq_copies(0):
        c.start(priority=0)
    for m in range(K_AHEAD):
        k_start(m)
    x_rest.start(priority=0)
    for n in range(V_AHEAD - RB):
        v_start(n)
    for c in wo_copies(0):
        c.start(priority=1)
    acc_s[...] = jnp.zeros(acc_s.shape, F32)
    wait_all([x_head] + wq_copies(0))
    for j in range(RB):
        q_piece(0, j)

    @pl.loop(0, RB)
    def _(j):
        step(-1, j, v_side=False, out_side=False)

    x_rest.wait()

    @pl.loop(0, RB)
    def _(j):
        step(0, j, out_side=False)

    wait_all(wo_copies(0))

    @pl.loop(1, NPH - 2)
    def _(ph):
        r, g = ph % NR, ph // NR

        @pl.when(jnp.logical_and(r == NR - 2, g < HKV - 1))
        def _():
            wait_all(wq_copies(g + 1))

        @pl.when(jnp.logical_and(r == 1, g > 0))
        def _():
            wait_all(wo_copies(g))

        @pl.when(jnp.logical_and(r == 1, g < HKV - 1))
        def _():
            start_split(wq_copies(g + 1))

        @pl.when(jnp.logical_and(r == 4, g < HKV - 1))
        def _():
            start_split(wo_copies(g + 1))

        @pl.loop(0, RB)
        def _(j):
            step(ph, j)

    A, Z = NPH - 2, NPH - 1
    n0 = A * RB

    k_wait(n0 + 4); v_wait(n0)
    attend(A, 0); s = scores(Z, 0); out_piece(A - 1, 0); out_piece(A - 1, 1); softmax(Z, 0, s)
    k_start(n0 + 7); v_start(n0 + 5)

    k_wait(n0 + 5); v_wait(n0 + 1)
    attend(A, 1); s = scores(Z, 1); out_piece(A - 1, 2); out_piece(A - 1, 3); softmax(Z, 1, s)
    v_start(n0 + 6)

    k_wait(n0 + 6); v_wait(n0 + 2)
    s = scores(Z, 2); attend(A, 2); softmax(Z, 2, s)
    v_start(n0 + 7)

    k_wait(n0 + 7); v_wait(n0 + 3)
    s = scores(Z, 3); attend(A, 3); softmax(Z, 3, s)

    v_wait(n0 + 4)
    attend(Z, 0)
    for j in range(RB):
        out_piece(A, j)

    v_wait(n0 + 5); v_wait(n0 + 6)
    attend(Z, 1); attend(Z, 2)

    v_wait(n0 + 7)
    early = [out_copy(0, Z % NR * RR - RR), out_copy(Z % NR * RR - RR, RR)]
    for c in early:
        c.start(priority=0)
    attend(Z, 3)
    out_piece(Z, 0, width=D)
    last = out_copy(Z % NR * RR, RR)
    last.start(priority=0)
    wait_all(early + [last])


def _call(x2d, k_cache, v_cache, wq, wo):
    return pl.pallas_call(
        _kernel,
        out_shape=jax.ShapeDtypeStruct((B * SQ, D), BF),
        in_specs=[pl.BlockSpec(memory_space=pl.ANY)] * 5,
        out_specs=pl.BlockSpec(memory_space=pl.ANY),
        scratch_shapes=[
            pltpu.VMEM((B * SQ, D), BF),
            pltpu.VMEM((D, HQ * DH), BF),
            pltpu.VMEM((HQ * DH, D), BF),
            pltpu.VMEM((NKB, SK, DH), BF),
            pltpu.VMEM((NVB, SK, DH), BF),
            pltpu.VMEM((2, RB, REP * SQ, DH), BF),
            pltpu.VMEM((2, RB, REP * SQ, SK), BF),
            pltpu.VMEM((2, RB, REP * SQ, DH), F32),
            pltpu.VMEM((2, RR, GW), BF),
            pltpu.VMEM((B * SQ, D), F32),
            pltpu.VMEM((B * SQ, D), BF),
            pltpu.SemaphoreType.DMA((NKB,)),
            pltpu.SemaphoreType.DMA((NVB,)),
            pltpu.SemaphoreType.DMA(()),
            pltpu.SemaphoreType.DMA(()),
            pltpu.SemaphoreType.DMA(()),
        ],
        compiler_params=pltpu.CompilerParams(vmem_limit_bytes=64 * 1024 * 1024,
                                             disable_bounds_checks=True),
        name="gqa_block_cached",
    )(x2d, k_cache, v_cache, wq, wo)


@jax.jit
def pallas_standalone__gqa_block_cached__sampling_kernel(
    x: jax.Array,
    k_cache: jax.Array,
    v_cache: jax.Array,
    wq: jax.Array,
    wo: jax.Array,
):
    out = _call(x.reshape(B * SQ, D), k_cache, v_cache, wq, wo)
    return out.reshape(B, SQ, D)
```

```python
import math

import jax
import jax.numpy as jnp
from jax import lax
from jax.experimental import pallas as pl
from jax.experimental.pallas import tpu as pltpu

B, SQ, D = 32, 16, 1024
HQ, HKV, SK, DH = 32, 4, 2048, 128
REP = HQ // HKV
GW = REP * DH
RB = 4
RR = RB * SQ
NR = B // RB
NPH = NR * HKV
NBLK = B * HKV
PW = GW // RB
HP = PW // DH

K_AHEAD = 3
V_AHEAD = 5
NKB = K_AHEAD + 1
NVB = V_AHEAD + 1
KV_CHUNKS = (192,) * 10 + (128,)

BF = jnp.bfloat16
F32 = jnp.float32
QSCALE = float(DH ** -0.5 * math.log2(math.e))

assert sum(KV_CHUNKS) == SK and NKB == 4 and RB == 4


def _aligned(v, m):
    return v if isinstance(v, int) else pl.multiple_of(v, m)


def _kernel(x_hbm, k_hbm, v_hbm, wq_hbm, wo_hbm, out_hbm,
            x_s, wq_s, wo_s, kbuf, vbuf, q_s, p_s, il_s, o_s, acc_s, out_s,
            sem_k, sem_v, sem_a, sem_b, sem_c):

    def block_start(hbm, buf, sem, n, ring, queue):
        off = 0
        for rows in KV_CHUNKS:
            pltpu.make_async_copy(hbm.at[n % B, n // B, pl.ds(off, rows)],
                                  buf.at[n % ring, pl.ds(off, rows)],
                                  sem.at[n % ring]).start(priority=queue)
            off += rows

    def block_wait(buf, sem, n, ring):
        pltpu.make_async_copy(buf.at[n % ring], buf.at[n % ring], sem.at[n % ring]).wait()

    def k_start(n):
        block_start(k_hbm, kbuf, sem_k, n, NKB, 0)

    def v_start(n):
        block_start(v_hbm, vbuf, sem_v, n, NVB, 1)

    def k_wait(n):
        block_wait(kbuf, sem_k, n, NKB)

    def v_wait(n):
        block_wait(vbuf, sem_v, n, NVB)

    def wq_copies(g):
        c0 = _aligned(g * GW, GW)
        return [pltpu.make_async_copy(wq_hbm.at[pl.ds(h * 512, 512), pl.ds(c0, GW)],
                                      wq_s.at[pl.ds(h * 512, 512), pl.ds(c0, GW)], sem_a)
                for h in range(2)]

    def wo_copies(g):
        return [pltpu.make_async_copy(wo_hbm.at[pl.ds(_aligned(g * GW + h * 512, 512), 512)],
                                      wo_s.at[pl.ds(_aligned(g * GW + h * 512, 512), 512)], sem_c)
                for h in range(2)]

    SLAB = GW // NR

    def wq_slab(g, i):
        rows, cols = pl.ds(_aligned(i * SLAB, SLAB), SLAB), pl.ds(_aligned(g * GW, GW), GW)
        return pltpu.make_async_copy(wq_hbm.at[rows, cols], wq_s.at[rows, cols], sem_a)

    def wo_slab(g, i):
        rows = pl.ds(_aligned(g * GW + i * SLAB, SLAB), SLAB)
        return pltpu.make_async_copy(wo_hbm.at[rows], wo_s.at[rows], sem_c)

    def wq_wait(g):
        cols = pl.ds(_aligned(g * GW, GW), GW)
        pltpu.make_async_copy(wq_s.at[:, cols], wq_s.at[:, cols], sem_a).wait()

    def wo_wait(g):
        rows = pl.ds(_aligned(g * GW, GW), GW)
        pltpu.make_async_copy(wo_s.at[rows], wo_s.at[rows], sem_c).wait()

    def wait_all(copies):
        for c in copies:
            c.wait()

    def out_copy(r0, rows):
        return pltpu.make_async_copy(out_s.at[pl.ds(r0, rows)], out_hbm.at[pl.ds(r0, rows)], sem_b)

    def q_piece(ph, j):
        g, r = ph // NR, ph % NR
        xs = x_s[pl.ds(_aligned(r * RR, RR), RR), :]
        w = wq_s[:, pl.ds(_aligned(g * GW + j * PW, PW), PW)]
        q = (jnp.dot(xs, w, preferred_element_type=F32) * QSCALE).astype(BF)
        for bl in range(RB):
            for t in range(HP):
                q_s[ph % 2, bl, pl.ds(_aligned((j * HP + t) * SQ, SQ), SQ), :] = (
                    q[bl * SQ:(bl + 1) * SQ, t * DH:(t + 1) * DH])

    def scores(ph, j):
        return lax.dot_general(q_s[ph % 2, j], kbuf[(ph * RB + j) % NKB],
                               (((1,), (1,)), ((), ())), preferred_element_type=F32)

    def softmax(ph, j, s):
        m = jnp.max(s, axis=-1, keepdims=True)
        p = jnp.exp2(s - m)
        l = jnp.sum(p, axis=-1, keepdims=True)
        p_s[ph % 2, j] = p.astype(BF)
        il_s[ph % 2, j] = jnp.broadcast_to(1.0 / l, (GW // DH * SQ, DH))

    def attend(ph, j):
        o = jnp.dot(p_s[ph % 2, j], vbuf[(ph * RB + j) % NVB], preferred_element_type=F32)
        o = (o * il_s[ph % 2, j]).astype(BF)
        for h in range(REP):
            o_s[ph % 2, pl.ds(_aligned(j * SQ, SQ), SQ), h * DH:(h + 1) * DH] = o[h * SQ:(h + 1) * SQ]

    def out_piece(ph, j, width=PW):
        g, r = ph // NR, ph % NR
        cols = pl.ds(_aligned(j * width, width), width)
        rows = pl.ds(_aligned(r * RR, RR), RR)
        res = jnp.dot(o_s[ph % 2], wo_s[pl.ds(_aligned(g * GW, GW), GW), cols],
                      preferred_element_type=F32) + acc_s[rows, cols]
        acc_s[rows, cols] = res
        out_s[rows, cols] = res.astype(BF)

    def step(ph, j, v_side=True, out_side=True):
        n = ph * RB + j
        k_wait(n + RB)
        if v_side:
            v_wait(n)
            attend(ph, j)
        s = scores(ph + 1, j)
        if out_side:
            out_piece(ph - 1, j)
        q_piece(ph + 2, j)
        softmax(ph + 1, j, s)
        k_start(n + RB + K_AHEAD)
        v_start(n + V_AHEAD)

    x_head = pltpu.make_async_copy(x_hbm.at[pl.ds(0, 2 * RR)], x_s.at[pl.ds(0, 2 * RR)], sem_a)
    x_rest = pltpu.make_async_copy(x_hbm.at[pl.ds(2 * RR, B * SQ - 2 * RR)],
                                   x_s.at[pl.ds(2 * RR, B * SQ - 2 * RR)], sem_b)
    x_head.start(priority=0)
    for c in wq_copies(0):
        c.start(priority=0)
    for m in range(K_AHEAD):
        k_start(m)
    x_rest.start(priority=0)
    for n in range(V_AHEAD - RB):
        v_start(n)
    for c in wo_copies(0):
        c.start(priority=1)
    acc_s[...] = jnp.zeros(acc_s.shape, F32)
    wait_all([x_head] + wq_copies(0))
    wq_slab(1, 0).start(priority=0)
    for j in range(RB):
        q_piece(0, j)
    wq_slab(1, 1).start(priority=0)

    @pl.loop(0, RB)
    def _(j):
        step(-1, j, v_side=False, out_side=False)

    x_rest.wait()
    wq_slab(1, 2).start(priority=0)

    @pl.loop(0, RB)
    def _(j):
        step(0, j, out_side=False)

    wait_all(wo_copies(0))

    @pl.loop(1, NPH - 2)
    def _(ph):
        r, g = ph % NR, ph // NR

        @pl.when(jnp.logical_and(r == NR - 2, g < HKV - 1))
        def _():
            wq_wait(g + 1)

        @pl.when(jnp.logical_and(r == 1, g > 0))
        def _():
            wo_wait(g)

        @pl.when(ph + 2 < (HKV - 1) * NR)
        def _():
            wq_slab((ph + 2) // NR + 1, (ph + 2) % NR).start(priority=0)

        @pl.when(ph + NR - 1 < HKV * NR)
        def _():
            wo_slab((ph + NR - 1) // NR, (ph + NR - 1) % NR).start(priority=1)

        @pl.loop(0, RB)
        def _(j):
            step(ph, j)

    A, Z = NPH - 2, NPH - 1
    n0 = A * RB

    k_wait(n0 + 4); v_wait(n0)
    attend(A, 0); s = scores(Z, 0); out_piece(A - 1, 0); out_piece(A - 1, 1); softmax(Z, 0, s)
    k_start(n0 + 7); v_start(n0 + 5)

    k_wait(n0 + 5); v_wait(n0 + 1)
    attend(A, 1); s = scores(Z, 1); out_piece(A - 1, 2); out_piece(A - 1, 3); softmax(Z, 1, s)
    v_start(n0 + 6)

    k_wait(n0 + 6); v_wait(n0 + 2)
    s = scores(Z, 2); attend(A, 2); softmax(Z, 2, s)
    v_start(n0 + 7)

    k_wait(n0 + 7); v_wait(n0 + 3)
    s = scores(Z, 3); attend(A, 3); softmax(Z, 3, s)

    v_wait(n0 + 4)
    attend(Z, 0)
    for j in range(RB):
        out_piece(A, j)

    v_wait(n0 + 5); v_wait(n0 + 6)
    attend(Z, 1); attend(Z, 2)

    v_wait(n0 + 7)
    early = [out_copy(0, Z % NR * RR - RR), out_copy(Z % NR * RR - RR, RR)]
    for c in early:
        c.start(priority=0)
    attend(Z, 3)
    out_piece(Z, 0, width=D)
    last = out_copy(Z % NR * RR, RR)
    last.start(priority=0)
    wait_all(early + [last])


def _call(x2d, k_cache, v_cache, wq, wo):
    return pl.pallas_call(
        _kernel,
        out_shape=jax.ShapeDtypeStruct((B * SQ, D), BF),
        in_specs=[pl.BlockSpec(memory_space=pl.ANY)] * 5,
        out_specs=pl.BlockSpec(memory_space=pl.ANY),
        scratch_shapes=[
            pltpu.VMEM((B * SQ, D), BF),
            pltpu.VMEM((D, HQ * DH), BF),
            pltpu.VMEM((HQ * DH, D), BF),
            pltpu.VMEM((NKB, SK, DH), BF),
            pltpu.VMEM((NVB, SK, DH), BF),
            pltpu.VMEM((2, RB, REP * SQ, DH), BF),
            pltpu.VMEM((2, RB, REP * SQ, SK), BF),
            pltpu.VMEM((2, RB, REP * SQ, DH), F32),
            pltpu.VMEM((2, RR, GW), BF),
            pltpu.VMEM((B * SQ, D), F32),
            pltpu.VMEM((B * SQ, D), BF),
            pltpu.SemaphoreType.DMA((NKB,)),
            pltpu.SemaphoreType.DMA((NVB,)),
            pltpu.SemaphoreType.DMA(()),
            pltpu.SemaphoreType.DMA(()),
            pltpu.SemaphoreType.DMA(()),
        ],
        compiler_params=pltpu.CompilerParams(vmem_limit_bytes=64 * 1024 * 1024,
                                             disable_bounds_checks=True),
        name="gqa_block_cached",
    )(x2d, k_cache, v_cache, wq, wo)


@jax.jit
def pallas_standalone__gqa_block_cached__sampling_kernel(
    x: jax.Array,
    k_cache: jax.Array,
    v_cache: jax.Array,
    wq: jax.Array,
    wo: jax.Array,
):
    out = _call(x.reshape(B * SQ, D), k_cache, v_cache, wq, wo)
    return out.reshape(B, SQ, D)
```

```python
import math

import jax
import jax.numpy as jnp
from jax import lax
from jax.experimental import pallas as pl
from jax.experimental.pallas import tpu as pltpu

B, SQ, D = 32, 16, 1024
HQ, HKV, SK, DH = 32, 4, 2048, 128
REP = HQ // HKV
GW = REP * DH
RB = 4
RR = RB * SQ
NR = B // RB
NPH = NR * HKV
NBLK = B * HKV
PW = GW // RB
HP = PW // DH

K_AHEAD = 3
V_AHEAD = 5
NKB = K_AHEAD + 1
NVB = V_AHEAD + 1
KV_CHUNKS = (192,) * 10 + (128,)
K_FIRST, V_FIRST = 6, 10

BF = jnp.bfloat16
F32 = jnp.float32
QSCALE = float(DH ** -0.5 * math.log2(math.e))

assert sum(KV_CHUNKS) == SK and NKB == 4 and RB == 4


def _aligned(v, m):
    return v if isinstance(v, int) else pl.multiple_of(v, m)


def _kernel(x_hbm, k_hbm, v_hbm, wq_hbm, wo_hbm, out_hbm,
            x_s, wq_s, wo_s, kbuf, vbuf, q_s, p_s, il_s, o_s, acc_s, out_s,
            sem_k, sem_v, sem_a, sem_b, sem_c):

    def block_start(hbm, buf, sem, n, ring, queue, first):
        for i in range(len(KV_CHUNKS)):
            c = (first + i) % len(KV_CHUNKS)
            off, rows = sum(KV_CHUNKS[:c]), KV_CHUNKS[c]
            pltpu.make_async_copy(hbm.at[n % B, n // B, pl.ds(off, rows)],
                                  buf.at[n % ring, pl.ds(off, rows)],
                                  sem.at[n % ring]).start(priority=queue)

    def block_wait(buf, sem, n, ring):
        pltpu.make_async_copy(buf.at[n % ring], buf.at[n % ring], sem.at[n % ring]).wait()

    def k_start(n):
        block_start(k_hbm, kbuf, sem_k, n, NKB, 0, K_FIRST)

    def v_start(n):
        block_start(v_hbm, vbuf, sem_v, n, NVB, 1, V_FIRST)

    def k_wait(n):
        block_wait(kbuf, sem_k, n, NKB)

    def v_wait(n):
        block_wait(vbuf, sem_v, n, NVB)

    def wq_copies(g):
        c0 = _aligned(g * GW, GW)
        return [pltpu.make_async_copy(wq_hbm.at[pl.ds(h * 512, 512), pl.ds(c0, GW)],
                                      wq_s.at[pl.ds(h * 512, 512), pl.ds(c0, GW)], sem_a)
                for h in range(2)]

    def wo_copies(g):
        return [pltpu.make_async_copy(wo_hbm.at[pl.ds(_aligned(g * GW + h * 512, 512), 512)],
                                      wo_s.at[pl.ds(_aligned(g * GW + h * 512, 512), 512)], sem_c)
                for h in range(2)]

    SLAB = GW // NR

    def wq_slab(g, i):
        rows, cols = pl.ds(_aligned(i * SLAB, SLAB), SLAB), pl.ds(_aligned(g * GW, GW), GW)
        return pltpu.make_async_copy(wq_hbm.at[rows, cols], wq_s.at[rows, cols], sem_a)

    def wo_slab(g, i):
        rows = pl.ds(_aligned(g * GW + i * SLAB, SLAB), SLAB)
        return pltpu.make_async_copy(wo_hbm.at[rows], wo_s.at[rows], sem_c)

    def wq_wait(g):
        cols = pl.ds(_aligned(g * GW, GW), GW)
        pltpu.make_async_copy(wq_s.at[:, cols], wq_s.at[:, cols], sem_a).wait()

    def wo_wait(g):
        rows = pl.ds(_aligned(g * GW, GW), GW)
        pltpu.make_async_copy(wo_s.at[rows], wo_s.at[rows], sem_c).wait()

    def wait_all(copies):
        for c in copies:
            c.wait()

    def out_copy(r0, rows):
        return pltpu.make_async_copy(out_s.at[pl.ds(r0, rows)], out_hbm.at[pl.ds(r0, rows)], sem_b)

    def q_piece(ph, j):
        g, r = ph // NR, ph % NR
        xs = x_s[pl.ds(_aligned(r * RR, RR), RR), :]
        w = wq_s[:, pl.ds(_aligned(g * GW + j * PW, PW), PW)]
        q = (jnp.dot(xs, w, preferred_element_type=F32) * QSCALE).astype(BF)
        for bl in range(RB):
            for t in range(HP):
                q_s[ph % 2, bl, pl.ds(_aligned((j * HP + t) * SQ, SQ), SQ), :] = (
                    q[bl * SQ:(bl + 1) * SQ, t * DH:(t + 1) * DH])

    def scores(ph, j):
        return lax.dot_general(q_s[ph % 2, j], kbuf[(ph * RB + j) % NKB],
                               (((1,), (1,)), ((), ())), preferred_element_type=F32)

    def softmax(ph, j, s):
        m = jnp.max(s, axis=-1, keepdims=True)
        p = jnp.exp2(s - m)
        l = jnp.sum(p, axis=-1, keepdims=True)
        p_s[ph % 2, j] = p.astype(BF)
        il_s[ph % 2, j] = jnp.broadcast_to(1.0 / l, (GW // DH * SQ, DH))

    def attend(ph, j):
        o = jnp.dot(p_s[ph % 2, j], vbuf[(ph * RB + j) % NVB], preferred_element_type=F32)
        o = (o * il_s[ph % 2, j]).astype(BF)
        for h in range(REP):
            o_s[ph % 2, pl.ds(_aligned(j * SQ, SQ), SQ), h * DH:(h + 1) * DH] = o[h * SQ:(h + 1) * SQ]

    def out_piece(ph, j, width=PW):
        g, r = ph // NR, ph % NR
        cols = pl.ds(_aligned(j * width, width), width)
        rows = pl.ds(_aligned(r * RR, RR), RR)
        res = jnp.dot(o_s[ph % 2], wo_s[pl.ds(_aligned(g * GW, GW), GW), cols],
                      preferred_element_type=F32) + acc_s[rows, cols]
        acc_s[rows, cols] = res
        out_s[rows, cols] = res.astype(BF)

    def step(ph, j, v_side=True, out_side=True):
        n = ph * RB + j
        k_wait(n + RB)
        if v_side:
            v_wait(n)
            attend(ph, j)
        s = scores(ph + 1, j)
        if out_side:
            out_piece(ph - 1, j)
        q_piece(ph + 2, j)
        softmax(ph + 1, j, s)
        k_start(n + RB + K_AHEAD)
        v_start(n + V_AHEAD)

    x_head = pltpu.make_async_copy(x_hbm.at[pl.ds(0, 2 * RR)], x_s.at[pl.ds(0, 2 * RR)], sem_a)
    x_rest = pltpu.make_async_copy(x_hbm.at[pl.ds(2 * RR, B * SQ - 2 * RR)],
                                   x_s.at[pl.ds(2 * RR, B * SQ - 2 * RR)], sem_b)
    x_head.start(priority=0)
    for c in wq_copies(0):
        c.start(priority=0)
    for m in range(K_AHEAD):
        k_start(m)
    x_rest.start(priority=0)
    for n in range(V_AHEAD - RB):
        v_start(n)
    for c in wo_copies(0):
        c.start(priority=1)
    acc_s[...] = jnp.zeros(acc_s.shape, F32)
    wait_all([x_head] + wq_copies(0))
    wq_slab(1, 0).start(priority=0)
    for j in range(RB):
        q_piece(0, j)
    wq_slab(1, 1).start(priority=0)

    @pl.loop(0, RB)
    def _(j):
        step(-1, j, v_side=False, out_side=False)

    x_rest.wait()
    wq_slab(1, 2).start(priority=0)

    @pl.loop(0, RB)
    def _(j):
        step(0, j, out_side=False)

    wait_all(wo_copies(0))

    @pl.loop(1, NPH - 2)
    def _(ph):
        r, g = ph % NR, ph // NR

        @pl.when(jnp.logical_and(r == NR - 2, g < HKV - 1))
        def _():
            wq_wait(g + 1)

        @pl.when(jnp.logical_and(r == 1, g > 0))
        def _():
            wo_wait(g)

        @pl.when(ph + 2 < (HKV - 1) * NR)
        def _():
            wq_slab((ph + 2) // NR + 1, (ph + 2) % NR).start(priority=0)

        @pl.when(ph + NR - 1 < HKV * NR)
        def _():
            wo_slab((ph + NR - 1) // NR, (ph + NR - 1) % NR).start(priority=1)

        @pl.loop(0, RB)
        def _(j):
            step(ph, j)

    A, Z = NPH - 2, NPH - 1
    n0 = A * RB

    k_wait(n0 + 4); v_wait(n0)
    attend(A, 0); s = scores(Z, 0); out_piece(A - 1, 0); out_piece(A - 1, 1); softmax(Z, 0, s)
    k_start(n0 + 7); v_start(n0 + 5)

    k_wait(n0 + 5); v_wait(n0 + 1)
    attend(A, 1); s = scores(Z, 1); out_piece(A - 1, 2); out_piece(A - 1, 3); softmax(Z, 1, s)
    v_start(n0 + 6)

    k_wait(n0 + 6); v_wait(n0 + 2)
    s = scores(Z, 2); attend(A, 2); softmax(Z, 2, s)
    v_start(n0 + 7)

    k_wait(n0 + 7); v_wait(n0 + 3)
    s = scores(Z, 3); attend(A, 3); softmax(Z, 3, s)

    v_wait(n0 + 4)
    attend(Z, 0)
    for j in range(RB):
        out_piece(A, j)

    v_wait(n0 + 5); v_wait(n0 + 6)
    attend(Z, 1); attend(Z, 2)

    v_wait(n0 + 7)
    early = [out_copy(0, Z % NR * RR - RR), out_copy(Z % NR * RR - RR, RR)]
    for c in early:
        c.start(priority=0)
    attend(Z, 3)
    out_piece(Z, 0, width=D)
    last = out_copy(Z % NR * RR, RR)
    last.start(priority=0)
    wait_all(early + [last])


def _call(x2d, k_cache, v_cache, wq, wo):
    return pl.pallas_call(
        _kernel,
        out_shape=jax.ShapeDtypeStruct((B * SQ, D), BF),
        in_specs=[pl.BlockSpec(memory_space=pl.ANY)] * 5,
        out_specs=pl.BlockSpec(memory_space=pl.ANY),
        scratch_shapes=[
            pltpu.VMEM((B * SQ, D), BF),
            pltpu.VMEM((D, HQ * DH), BF),
            pltpu.VMEM((HQ * DH, D), BF),
            pltpu.VMEM((NKB, SK, DH), BF),
            pltpu.VMEM((NVB, SK, DH), BF),
            pltpu.VMEM((2, RB, REP * SQ, DH), BF),
            pltpu.VMEM((2, RB, REP * SQ, SK), BF),
            pltpu.VMEM((2, RB, REP * SQ, DH), F32),
            pltpu.VMEM((2, RR, GW), BF),
            pltpu.VMEM((B * SQ, D), F32),
            pltpu.VMEM((B * SQ, D), BF),
            pltpu.SemaphoreType.DMA((NKB,)),
            pltpu.SemaphoreType.DMA((NVB,)),
            pltpu.SemaphoreType.DMA(()),
            pltpu.SemaphoreType.DMA(()),
            pltpu.SemaphoreType.DMA(()),
        ],
        compiler_params=pltpu.CompilerParams(vmem_limit_bytes=64 * 1024 * 1024,
                                             disable_bounds_checks=True),
        name="gqa_block_cached",
    )(x2d, k_cache, v_cache, wq, wo)


@jax.jit
def pallas_standalone__gqa_block_cached__sampling_kernel(
    x: jax.Array,
    k_cache: jax.Array,
    v_cache: jax.Array,
    wq: jax.Array,
    wo: jax.Array,
):
    out = _call(x.reshape(B * SQ, D), k_cache, v_cache, wq, wo)
    return out.reshape(B, SQ, D)
```

```python
import math

import jax
import jax.numpy as jnp
from jax import lax
from jax.experimental import pallas as pl
from jax.experimental.pallas import tpu as pltpu

B, SQ, D = 32, 16, 1024
HQ, HKV, SK, DH = 32, 4, 2048, 128
REP = HQ // HKV
GW = REP * DH
RB = 4
RR = RB * SQ
NR = B // RB
NPH = NR * HKV
NBLK = B * HKV
PW = GW // RB
HP = PW // DH

K_AHEAD = 3
V_AHEAD = 5
NKB = K_AHEAD + 1
NVB = V_AHEAD + 1
KV_CHUNKS = (192,) * 10 + (128,)
K_FIRST, V_FIRST = 6, 10

BF = jnp.bfloat16
F32 = jnp.float32
QSCALE = float(DH ** -0.5 * math.log2(math.e))

assert sum(KV_CHUNKS) == SK and NKB == 4 and RB == 4


def _aligned(v, m):
    return v if isinstance(v, int) else pl.multiple_of(v, m)


def _kernel(*refs):
    dma_sem = pltpu.SemaphoreType.DMA
    pl.run_scoped(lambda *sems: _body(*refs, *sems),
                  dma_sem((NKB,)), dma_sem((NVB,)), dma_sem(()), dma_sem(()), dma_sem(()))


def _body(x_hbm, k_hbm, v_hbm, wq_hbm, wo_hbm, out_hbm,
          x_s, wq_s, wo_s, kbuf, vbuf, q_s, p_s, il_s, o_s, acc_s, out_s,
          sem_k, sem_v, sem_a, sem_b, sem_c):

    def block_start(hbm, buf, sem, n, ring, queue, first):
        for i in range(len(KV_CHUNKS)):
            c = (first + i) % len(KV_CHUNKS)
            off, rows = sum(KV_CHUNKS[:c]), KV_CHUNKS[c]
            pltpu.make_async_copy(hbm.at[n % B, n // B, pl.ds(off, rows)],
                                  buf.at[n % ring, pl.ds(off, rows)],
                                  sem.at[n % ring]).start(priority=queue)

    def block_wait(buf, sem, n, ring):
        pltpu.make_async_copy(buf.at[n % ring], buf.at[n % ring], sem.at[n % ring]).wait()

    def k_start(n):
        block_start(k_hbm, kbuf, sem_k, n, NKB, 0, K_FIRST)

    def v_start(n):
        block_start(v_hbm, vbuf, sem_v, n, NVB, 1, V_FIRST)

    def k_wait(n):
        block_wait(kbuf, sem_k, n, NKB)

    def v_wait(n):
        block_wait(vbuf, sem_v, n, NVB)

    def wq_copies(g):
        c0 = _aligned(g * GW, GW)
        return [pltpu.make_async_copy(wq_hbm.at[pl.ds(h * 512, 512), pl.ds(c0, GW)],
                                      wq_s.at[pl.ds(h * 512, 512), pl.ds(c0, GW)], sem_a)
                for h in range(2)]

    def wo_copies(g):
        return [pltpu.make_async_copy(wo_hbm.at[pl.ds(_aligned(g * GW + h * 512, 512), 512)],
                                      wo_s.at[pl.ds(_aligned(g * GW + h * 512, 512), 512)], sem_c)
                for h in range(2)]

    SLAB = GW // NR

    def wq_slab(g, i):
        rows, cols = pl.ds(_aligned(i * SLAB, SLAB), SLAB), pl.ds(_aligned(g * GW, GW), GW)
        return pltpu.make_async_copy(wq_hbm.at[rows, cols], wq_s.at[rows, cols], sem_a)

    def wo_slab(g, i):
        rows = pl.ds(_aligned(g * GW + i * SLAB, SLAB), SLAB)
        return pltpu.make_async_copy(wo_hbm.at[rows], wo_s.at[rows], sem_c)

    def wq_wait(g):
        cols = pl.ds(_aligned(g * GW, GW), GW)
        pltpu.make_async_copy(wq_s.at[:, cols], wq_s.at[:, cols], sem_a).wait()

    def wo_wait(g):
        rows = pl.ds(_aligned(g * GW, GW), GW)
        pltpu.make_async_copy(wo_s.at[rows], wo_s.at[rows], sem_c).wait()

    def wait_all(copies):
        for c in copies:
            c.wait()

    def out_copy(r0, rows):
        return pltpu.make_async_copy(out_s.at[pl.ds(r0, rows)], out_hbm.at[pl.ds(r0, rows)], sem_b)

    def q_piece(ph, j):
        g, r = ph // NR, ph % NR
        xs = x_s[pl.ds(_aligned(r * RR, RR), RR), :]
        w = wq_s[:, pl.ds(_aligned(g * GW + j * PW, PW), PW)]
        q = (jnp.dot(xs, w, preferred_element_type=F32) * QSCALE).astype(BF)
        for bl in range(RB):
            for t in range(HP):
                q_s[ph % 2, bl, pl.ds(_aligned((j * HP + t) * SQ, SQ), SQ), :] = (
                    q[bl * SQ:(bl + 1) * SQ, t * DH:(t + 1) * DH])

    def scores(ph, j):
        return lax.dot_general(q_s[ph % 2, j], kbuf[(ph * RB + j) % NKB],
                               (((1,), (1,)), ((), ())), preferred_element_type=F32)

    def softmax(ph, j, s):
        m = jnp.max(s, axis=-1, keepdims=True)
        p = jnp.exp2(s - m)
        l = jnp.sum(p, axis=-1, keepdims=True)
        p_s[ph % 2, j] = p.astype(BF)
        il_s[ph % 2, j] = jnp.broadcast_to(1.0 / l, (GW // DH * SQ, DH))

    def attend(ph, j):
        o = jnp.dot(p_s[ph % 2, j], vbuf[(ph * RB + j) % NVB], preferred_element_type=F32)
        o = (o * il_s[ph % 2, j]).astype(BF)
        for h in range(REP):
            o_s[ph % 2, pl.ds(_aligned(j * SQ, SQ), SQ), h * DH:(h + 1) * DH] = o[h * SQ:(h + 1) * SQ]

    def out_piece(ph, j, width=PW):
        g, r = ph // NR, ph % NR
        cols = pl.ds(_aligned(j * width, width), width)
        rows = pl.ds(_aligned(r * RR, RR), RR)
        res = jnp.dot(o_s[ph % 2], wo_s[pl.ds(_aligned(g * GW, GW), GW), cols],
                      preferred_element_type=F32) + acc_s[rows, cols]
        acc_s[rows, cols] = res
        out_s[rows, cols] = res.astype(BF)

    def step(ph, j, v_side=True, out_side=True):
        n = ph * RB + j
        k_wait(n + RB)
        if v_side:
            v_wait(n)
            attend(ph, j)
        s = scores(ph + 1, j)
        if out_side:
            out_piece(ph - 1, j)
        q_piece(ph + 2, j)
        softmax(ph + 1, j, s)
        k_start(n + RB + K_AHEAD)
        v_start(n + V_AHEAD)

    x_head = pltpu.make_async_copy(x_hbm.at[pl.ds(0, 2 * RR)], x_s.at[pl.ds(0, 2 * RR)], sem_a)
    x_rest = pltpu.make_async_copy(x_hbm.at[pl.ds(2 * RR, B * SQ - 2 * RR)],
                                   x_s.at[pl.ds(2 * RR, B * SQ - 2 * RR)], sem_b)
    x_head.start(priority=0)
    for c in wq_copies(0):
        c.start(priority=0)
    for m in range(K_AHEAD):
        k_start(m)
    x_rest.start(priority=0)
    for n in range(V_AHEAD - RB):
        v_start(n)
    for c in wo_copies(0):
        c.start(priority=1)
    acc_s[...] = jnp.zeros(acc_s.shape, F32)
    wait_all([x_head] + wq_copies(0))
    wq_slab(1, 0).start(priority=0)
    for j in range(RB):
        q_piece(0, j)
    wq_slab(1, 1).start(priority=0)

    @pl.loop(0, RB)
    def _(j):
        step(-1, j, v_side=False, out_side=False)

    x_rest.wait()
    wq_slab(1, 2).start(priority=0)

    @pl.loop(0, RB)
    def _(j):
        step(0, j, out_side=False)

    wait_all(wo_copies(0))

    @pl.loop(1, NPH - 2)
    def _(ph):
        r, g = ph % NR, ph // NR

        @pl.when(jnp.logical_and(r == NR - 2, g < HKV - 1))
        def _():
            wq_wait(g + 1)

        @pl.when(jnp.logical_and(r == 1, g > 0))
        def _():
            wo_wait(g)

        @pl.when(ph + 2 < (HKV - 1) * NR)
        def _():
            wq_slab((ph + 2) // NR + 1, (ph + 2) % NR).start(priority=0)

        @pl.when(ph + NR - 1 < HKV * NR)
        def _():
            wo_slab((ph + NR - 1) // NR, (ph + NR - 1) % NR).start(priority=1)

        @pl.loop(0, RB)
        def _(j):
            step(ph, j)

    A, Z = NPH - 2, NPH - 1
    n0 = A * RB

    k_wait(n0 + 4); v_wait(n0)
    attend(A, 0); s = scores(Z, 0); out_piece(A - 1, 0); out_piece(A - 1, 1); softmax(Z, 0, s)
    k_start(n0 + 7); v_start(n0 + 5)

    k_wait(n0 + 5); v_wait(n0 + 1)
    attend(A, 1); s = scores(Z, 1); out_piece(A - 1, 2); out_piece(A - 1, 3); softmax(Z, 1, s)
    v_start(n0 + 6)

    k_wait(n0 + 6); v_wait(n0 + 2)
    s = scores(Z, 2); attend(A, 2); softmax(Z, 2, s)
    v_start(n0 + 7)

    k_wait(n0 + 7); v_wait(n0 + 3)
    s = scores(Z, 3); attend(A, 3); softmax(Z, 3, s)

    v_wait(n0 + 4)
    attend(Z, 0)
    for j in range(RB):
        out_piece(A, j)

    v_wait(n0 + 5); v_wait(n0 + 6)
    attend(Z, 1); attend(Z, 2)

    v_wait(n0 + 7)
    early = [out_copy(0, Z % NR * RR - RR), out_copy(Z % NR * RR - RR, RR)]
    for c in early:
        c.start(priority=0)
    attend(Z, 3)
    out_piece(Z, 0, width=D)
    last = out_copy(Z % NR * RR, RR)
    last.start(priority=0)
    wait_all(early + [last])


def _call(x2d, k_cache, v_cache, wq, wo):
    return pl.pallas_call(
        _kernel,
        out_shape=jax.ShapeDtypeStruct((B * SQ, D), BF),
        in_specs=[pl.BlockSpec(memory_space=pl.ANY)] * 5,
        out_specs=pl.BlockSpec(memory_space=pl.ANY),
        scratch_shapes=[
            pltpu.VMEM((B * SQ, D), BF),
            pltpu.VMEM((D, HQ * DH), BF),
            pltpu.VMEM((HQ * DH, D), BF),
            pltpu.VMEM((NKB, SK, DH), BF),
            pltpu.VMEM((NVB, SK, DH), BF),
            pltpu.VMEM((2, RB, REP * SQ, DH), BF),
            pltpu.VMEM((2, RB, REP * SQ, SK), BF),
            pltpu.VMEM((2, RB, REP * SQ, DH), F32),
            pltpu.VMEM((2, RR, GW), BF),
            pltpu.VMEM((B * SQ, D), F32),
            pltpu.VMEM((B * SQ, D), BF),
        ],
        compiler_params=pltpu.CompilerParams(vmem_limit_bytes=64 * 1024 * 1024,
                                             disable_bounds_checks=True),
        name="gqa_block_cached",
    )(x2d, k_cache, v_cache, wq, wo)


@jax.jit
def pallas_standalone__gqa_block_cached__sampling_kernel(
    x: jax.Array,
    k_cache: jax.Array,
    v_cache: jax.Array,
    wq: jax.Array,
    wo: jax.Array,
):
    out = _call(x.reshape(B * SQ, D), k_cache, v_cache, wq, wo)
    return out.reshape(B, SQ, D)
```

```python
import math

import jax
import jax.numpy as jnp
from jax import lax
from jax.experimental import pallas as pl
from jax.experimental.pallas import tpu as pltpu

B, SQ, D = 32, 16, 1024
HQ, HKV, SK, DH = 32, 4, 2048, 128
REP = HQ // HKV
GW = REP * DH
RB = 4
RR = RB * SQ
NR = B // RB
NPH = NR * HKV
NBLK = B * HKV
PW = GW // RB
HP = PW // DH

K_AHEAD = 3
V_AHEAD = 5
NKB = K_AHEAD + 1
NVB = V_AHEAD + 1
KV_CHUNKS = (192,) * 10 + (128,)
K_FIRST, V_FIRST = 6, 10
WROWS = 16
SLAB = GW // NR

BF = jnp.bfloat16
F32 = jnp.float32
QSCALE = float(DH ** -0.5 * math.log2(math.e))

assert sum(KV_CHUNKS) == SK and (RB, K_AHEAD, V_AHEAD) == (4, 3, 5)


def _aligned(v, m):
    return v if isinstance(v, int) else pl.multiple_of(v, m)


def _kernel(*refs):
    dma_sem = pltpu.SemaphoreType.DMA
    pl.run_scoped(lambda *sems: _body(*refs, *sems), dma_sem((NKB + NVB,)),
                  dma_sem(()), dma_sem(()), dma_sem(()), dma_sem(()))


def _body(x_hbm, k_hbm, v_hbm, wq_hbm, wo_hbm, out_hbm,
          x_s, wq_s, wo_s, kbuf, vbuf, q_s, p_s, il_s, o_s, acc_s, out_s,
          sem_kv, sem_x, sem_wq, sem_wo, sem_out):

    def k_sem(n):
        return sem_kv.at[n % NKB]

    def v_sem(n):
        return sem_kv.at[NKB + n % NVB]

    def kv_start(k=None, v=None):
        for i in range(len(KV_CHUNKS)):
            for n, hbm, buf, ring, sem, queue, first in ((k, k_hbm, kbuf, NKB, k_sem, 0, K_FIRST),
                                                         (v, v_hbm, vbuf, NVB, v_sem, 1, V_FIRST)):
                if n is not None:
                    c = (first + i) % len(KV_CHUNKS)
                    rows = pl.ds(sum(KV_CHUNKS[:c]), KV_CHUNKS[c])
                    pltpu.make_async_copy(hbm.at[n % B, n // B, rows], buf.at[n % ring, rows],
                                          sem(n)).start(priority=queue)

    def wait_filled(buf, sem):
        pltpu.make_async_copy(buf, buf, sem).wait()

    def k_wait(n):
        wait_filled(kbuf.at[n % NKB], k_sem(n))

    def v_wait(n):
        wait_filled(vbuf.at[n % NVB], v_sem(n))

    def wq_start(g, r0, rows, queue):
        rs, cs = pl.ds(_aligned(r0, WROWS), rows), pl.ds(_aligned(g * GW, GW), GW)
        pltpu.make_async_copy(wq_hbm.at[rs, cs], wq_s.at[rs, cs], sem_wq).start(priority=queue)

    def wo_start(g, r0, rows, queue):
        rs = pl.ds(_aligned(g * GW + r0, WROWS), rows)
        pltpu.make_async_copy(wo_hbm.at[rs], wo_s.at[rs], sem_wo).start(priority=queue)

    def wq_wait(g):
        wait_filled(wq_s.at[:, pl.ds(_aligned(g * GW, GW), GW)], sem_wq)

    def wo_wait(g):
        wait_filled(wo_s.at[pl.ds(_aligned(g * GW, GW), GW)], sem_wo)

    def out_copy(r0, rows):
        return pltpu.make_async_copy(out_s.at[pl.ds(r0, rows)], out_hbm.at[pl.ds(r0, rows)], sem_out)

    def q_piece(ph, j):
        g, r = ph // NR, ph % NR
        xs = x_s[pl.ds(_aligned(r * RR, RR), RR), :]
        w = wq_s[:, pl.ds(_aligned(g * GW + j * PW, PW), PW)]
        q = (jnp.dot(xs, w, preferred_element_type=F32) * QSCALE).astype(BF)
        for bl in range(RB):
            for t in range(HP):
                q_s[ph % 2, bl, pl.ds(_aligned((j * HP + t) * SQ, SQ), SQ), :] = (
                    q[bl * SQ:(bl + 1) * SQ, t * DH:(t + 1) * DH])

    def scores(ph, j):
        return lax.dot_general(q_s[ph % 2, j], kbuf[(ph * RB + j) % NKB],
                               (((1,), (1,)), ((), ())), preferred_element_type=F32)

    def softmax(ph, j, s):
        m = jnp.max(s, axis=-1, keepdims=True)
        p = jnp.exp2(s - m)
        l = jnp.sum(p, axis=-1, keepdims=True)
        p_s[ph % 2, j] = p.astype(BF)
        il_s[ph % 2, j] = jnp.broadcast_to(1.0 / l, (REP * SQ, DH))

    def attend(ph, j):
        o = jnp.dot(p_s[ph % 2, j], vbuf[(ph * RB + j) % NVB], preferred_element_type=F32)
        o = (o * il_s[ph % 2, j]).astype(BF)
        for h in range(REP):
            o_s[ph % 2, pl.ds(_aligned(j * SQ, SQ), SQ), h * DH:(h + 1) * DH] = o[h * SQ:(h + 1) * SQ]

    def out_piece(ph, j, width=PW):
        g, r = ph // NR, ph % NR
        cols = pl.ds(_aligned(j * width, width), width)
        rows = pl.ds(_aligned(r * RR, RR), RR)
        res = jnp.dot(o_s[ph % 2], wo_s[pl.ds(_aligned(g * GW, GW), GW), cols],
                      preferred_element_type=F32) + acc_s[rows, cols]
        acc_s[rows, cols] = res
        out_s[rows, cols] = res.astype(BF)

    def step(ph, j, v_side=True, out_side=True):
        n = ph * RB + j
        k_wait(n + RB)
        if v_side:
            v_wait(n)
            attend(ph, j)
        s = scores(ph + 1, j)
        if out_side:
            out_piece(ph - 1, j)
        q_piece(ph + 2, j)
        softmax(ph + 1, j, s)
        kv_start(n + RB + K_AHEAD, n + V_AHEAD)

    @pl.loop(0, B * SQ // (2 * WROWS))
    def _(i):
        for queue in range(2):
            rs = pl.ds(pl.multiple_of((2 * i + queue) * WROWS, WROWS), WROWS)
            pltpu.make_async_copy(x_hbm.at[rs], x_s.at[rs], sem_x).start(priority=queue)

    @pl.loop(0, GW // WROWS)
    def _(i):
        wq_start(0, i * WROWS, WROWS, 0)
        wo_start(0, i * WROWS, WROWS, 1)

    kv_start(0, 0)
    for m in range(1, K_AHEAD):
        kv_start(m, None)
    acc_s[...] = jnp.zeros(acc_s.shape, F32)
    wait_filled(x_s, sem_x)
    wq_wait(0)
    for i in range(3):
        wq_start(1, i * SLAB, SLAB, 1)
    for j in range(RB):
        q_piece(0, j)

    @pl.loop(0, RB)
    def _(j):
        step(-1, j, v_side=False, out_side=False)

    @pl.loop(0, RB)
    def _(j):
        step(0, j, out_side=False)

    wo_wait(0)

    @pl.loop(1, NPH - 2)
    def _(ph):
        r, g = ph % NR, ph // NR

        @pl.when(jnp.logical_and(r == NR - 2, g < HKV - 1))
        def _():
            wq_wait(g + 1)

        @pl.when(jnp.logical_and(r == 1, g > 0))
        def _():
            wo_wait(g)

        tq, to = ph + 2, ph + NR - 1

        @pl.when(tq < (HKV - 1) * NR)
        def _():
            for u in range(SLAB // WROWS):
                wq_start(tq // NR + 1, (tq % NR) * SLAB + u * WROWS, WROWS, 0)
                wo_start(to // NR, (to % NR) * SLAB + u * WROWS, WROWS, 1)

        @pl.when(jnp.logical_and(tq >= (HKV - 1) * NR, to < HKV * NR))
        def _():
            for u in range(SLAB // WROWS):
                wo_start(to // NR, (to % NR) * SLAB + u * WROWS, WROWS, u % 2)

        @pl.loop(0, RB)
        def _(j):
            step(ph, j)

    A, Z = NPH - 2, NPH - 1
    n0 = A * RB

    k_wait(n0 + 4); v_wait(n0)
    attend(A, 0); s = scores(Z, 0); out_piece(A - 1, 0); out_piece(A - 1, 1); softmax(Z, 0, s)
    kv_start(n0 + 7, n0 + 5)

    k_wait(n0 + 5); v_wait(n0 + 1)
    attend(A, 1); s = scores(Z, 1); out_piece(A - 1, 2); out_piece(A - 1, 3); softmax(Z, 1, s)
    kv_start(None, n0 + 6)

    k_wait(n0 + 6); v_wait(n0 + 2)
    s = scores(Z, 2); attend(A, 2); softmax(Z, 2, s)
    kv_start(None, n0 + 7)

    k_wait(n0 + 7); v_wait(n0 + 3)
    s = scores(Z, 3); attend(A, 3); softmax(Z, 3, s)

    v_wait(n0 + 4)
    attend(Z, 0)
    for j in range(RB):
        out_piece(A, j)

    v_wait(n0 + 5); v_wait(n0 + 6)
    out_copy(0, RR).start(priority=1)
    attend(Z, 1); attend(Z, 2)

    v_wait(n0 + 7)
    out_copy(RR, (NR - 3) * RR).start(priority=0)
    out_copy((NR - 2) * RR, RR).start(priority=0)
    attend(Z, 3)
    out_piece(Z, 0, width=D)
    out_copy((NR - 1) * RR, RR).start(priority=0)
    pltpu.make_async_copy(out_s, out_hbm, sem_out).wait()


def _call(x2d, k_cache, v_cache, wq, wo):
    return pl.pallas_call(
        _kernel,
        out_shape=jax.ShapeDtypeStruct((B * SQ, D), BF),
        in_specs=[pl.BlockSpec(memory_space=pl.ANY)] * 5,
        out_specs=pl.BlockSpec(memory_space=pl.ANY),
        scratch_shapes=[
            pltpu.VMEM((B * SQ, D), BF),
            pltpu.VMEM((D, HQ * DH), BF),
            pltpu.VMEM((HQ * DH, D), BF),
            pltpu.VMEM((NKB, SK, DH), BF),
            pltpu.VMEM((NVB, SK, DH), BF),
            pltpu.VMEM((2, RB, REP * SQ, DH), BF),
            pltpu.VMEM((2, RB, REP * SQ, SK), BF),
            pltpu.VMEM((2, RB, REP * SQ, DH), F32),
            pltpu.VMEM((2, RR, GW), BF),
            pltpu.VMEM((B * SQ, D), F32),
            pltpu.VMEM((B * SQ, D), BF),
        ],
        compiler_params=pltpu.CompilerParams(vmem_limit_bytes=64 * 1024 * 1024,
                                             disable_bounds_checks=True),
        name="gqa_block_cached",
    )(x2d, k_cache, v_cache, wq, wo)


@jax.jit
def pallas_standalone__gqa_block_cached__sampling_kernel(
    x: jax.Array,
    k_cache: jax.Array,
    v_cache: jax.Array,
    wq: jax.Array,
    wo: jax.Array,
):
    out = _call(x.reshape(B * SQ, D), k_cache, v_cache, wq, wo)
    return out.reshape(B, SQ, D)
```
